```python
import os as _os
_os.environ.setdefault("JAX_PLATFORMS", "cpu")
import jax
import jax.numpy as jnp

def _softmax(x, axis=-1):
    return jax.nn.softmax(x, axis=axis)
def _gelu(x):
    return jax.nn.gelu(x, approximate=True)
def _silu(x):
    return jax.nn.silu(x)
def _sigmoid(x):
    return jax.nn.sigmoid(x)
def _layernorm(x, axis=-1, eps=1e-5):
    m = jnp.mean(x, axis=axis, keepdims=True)
    v = jnp.var(x, axis=axis, keepdims=True)
    return (x - m) / jnp.sqrt(v + eps)
def _scatter_add(tgt, idx, src, axis=0):
    return tgt.at[idx].add(src)
def _segment_sum(src, seg, n):
    return jax.ops.segment_sum(src, seg, n)
class _Rng:
    def __init__(self, key):
        self._k = key
    def _next(self):
        self._k, sub = jax.random.split(self._k)
        return sub
    def normal(self, shape):
        return jax.random.normal(self._next(), shape, dtype=jnp.bfloat16)
    def randint(self, lo, hi, shape):
        return jax.random.randint(self._next(), shape, lo, hi, dtype=jnp.int32)
    def uniform(self, shape, lo=0.0, hi=1.0):
        return jax.random.uniform(self._next(), shape, jnp.bfloat16, lo, hi)
    def permutation(self, n):
        return jax.random.permutation(self._next(), n)


kernel_name = 'gated_mix__mha_block__dense_activation_mish__prompt'

def setup_inputs():
    _rng = _Rng(jax.random.key(int.from_bytes(__import__("os").urandom(4), "little")))
    _w = (lambda a: (lambda t: t.astype(jnp.bfloat16) if jnp.issubdtype(t.dtype, jnp.floating) else t)(jnp.asarray(a)))
    def _A_setup():
        B, S, D, H = 1, 2048, 640, 32
        return {
            "x": _w((lambda *s: _rng.normal(s) * 0.05)(B, S, D)),
            "wqkv": _w((lambda *s: _rng.normal(s) * 0.2)(D, 3 * D)),
            "wo": _w((lambda *s: _rng.normal(s) * 0.05)(D, D)),
        }
    _A_in = _A_setup()

    def _B_setup():
        B, S, D, F = 1, 2048, 640, 1536
        return {
            "x": _w((lambda *s: _rng.normal(s) * 0.05)(B, S, D)),
            "w1": _w((lambda *s: _rng.normal(s) * 0.8)(D, F) * (D ** -0.5)),
            "b1": _w((lambda *s: _rng.normal(s) * 0.05)(F)),
            "w2": _w((lambda *s: _rng.normal(s) * 0.05)(F, D) * (F ** -0.5)),
        }
    _B_in = _B_setup()

    return {
        "A_x": _A_in["x"],
        "A_wqkv": _A_in["wqkv"],
        "A_wo": _A_in["wo"],
        "B_x": _B_in["x"],
        "B_w1": _B_in["w1"],
        "B_b1": _B_in["b1"],
        "B_w2": _B_in["w2"],
        "gate_w": _w((lambda *s: _rng.normal(s) * 0.05)(640) * 16.0),
    }

def reference(A_x, A_wqkv, A_wo, B_x, B_w1, B_b1, B_w2, gate_w):
    def _A_ref(x, wqkv, wo):
        B, S, D = x.shape
        H = 32
        Dh = D // H
        qkv = (lambda x, *d: x.transpose(*d))((x @ wqkv).reshape(B, S, 3, H, Dh), 2, 0, 3, 1, 4)
        q, k, v = qkv[0], qkv[1], qkv[2]
        scores = jnp.einsum("bhqd,bhkd->bhqk", q, k) * (Dh ** -0.5)
        p = _softmax(scores, axis=-1)
        o = jnp.einsum("bhqk,bhkd->bhqd", p, v)
        return (lambda x, *d: x.transpose(*d))(o, 0, 2, 1, 3).reshape(B, S, D) @ wo

    def _B_ref(x, w1, b1, w2):
        h = jnp.einsum("bsd,df->bsf", x, w1) + b1
        sp = jnp.log1p(jnp.exp(-jnp.abs(h))) + jnp.where(h > 0, h, jnp.zeros_like(h))
        act = h * jnp.tanh(sp)
        return jnp.einsum("bsf,fd->bsd", act, w2)

    x = A_x
    g = _sigmoid((x * gate_w).sum(-1, keepdims=True))
    a = _A_ref(x, A_wqkv, A_wo)
    b = _B_ref(x, B_w1, B_b1, B_w2)
    return g * a + (1 - g) * b
```

```python
import functools
import jax
import jax.numpy as jnp
import numpy as np
from jax import lax
from jax.experimental import pallas as pl
from jax.experimental.pallas import tpu as pltpu


S, D, H, DH, F = 2048, 640, 32, 20, 1536
NQ = 512
RB = 512
HB = 4
LOG2E = 1.4426950408889634
QSCALE = DH ** -0.5 * LOG2E
NT = (((1,), (1,)), ((), ()))
SAFE_LOG2 = 48.0


def _mish(h):
    e = jnp.exp(jnp.minimum(h, 20.0))
    n = e * (e + 2.0)
    return h * n / (n + 2.0)


def kernel(x_hbm, wqkv_hbm, wo_hbm, w1_hbm, b1_ref, w2_hbm, gw_ref, out_hbm,
           x_v, wqkv_v, wo_v, w1_v, w2_v, k_s, q_s, vt_s, ot_s, ob_s, sems, osem):
    f32, bf16 = jnp.float32, jnp.bfloat16
    nrb = S // RB
    cp_x = [pltpu.make_async_copy(x_hbm.at[pl.ds(i * RB, RB)], x_v.at[pl.ds(i * RB, RB)], sems.at[i]) for i in range(nrb)]
    cp_wqkv = pltpu.make_async_copy(wqkv_hbm, wqkv_v, sems.at[nrb])
    cp_w1 = pltpu.make_async_copy(w1_hbm, w1_v, sems.at[nrb + 1])
    cp_w2 = pltpu.make_async_copy(w2_hbm, w2_v, sems.at[nrb + 2])
    cp_wo = pltpu.make_async_copy(wo_hbm, wo_v, sems.at[nrb + 3])
    cp_x[0].start()
    cp_wqkv.start()
    for i in range(1, nrb):
        cp_x[i].start()
    cp_w1.start(); cp_w2.start(); cp_wo.start()

    lane = lax.broadcasted_iota(jnp.int32, (RB, 128), 1)
    row8 = lax.broadcasted_iota(jnp.int32, (8, RB), 0)

    cp_wqkv.wait()

    def ext_tiles(a):
        t = [a[:, 128 * i:128 * (i + 1)] for i in range(5)]
        return t + [jnp.where(lane >= 64, t[i], t[i + 1]) for i in range(4)]

    def proj_body(i, carry):
        qmax, kmax, vmax = carry
        off = pl.multiple_of(i * RB, RB)
        pltpu.make_async_copy(x_hbm.at[pl.ds(off, RB)], x_v.at[pl.ds(off, RB)], sems.at[i]).wait()
        xb = x_v[pl.ds(off, RB), :]
        k = jnp.dot(xb, wqkv_v[:, D:2 * D], preferred_element_type=f32)
        kb = k.astype(bf16)
        for t, tile in enumerate(ext_tiles(kb)):
            k_s[t, pl.ds(off, RB), :] = tile
        kmax = jnp.maximum(kmax, jnp.max(jnp.abs(kb.astype(f32)).reshape(RB // 8, 8, D), axis=0))
        q = jnp.dot(xb, wqkv_v[:, 0:D], preferred_element_type=f32) * QSCALE
        qb = q.astype(bf16)
        for t, tile in enumerate(ext_tiles(qb)):
            q_s[t, pl.ds(off, RB), :] = tile
        qmax = jnp.maximum(qmax, jnp.max(jnp.abs(qb.astype(f32)).reshape(RB // 8, 8, D), axis=0))
        v = jnp.dot(xb, wqkv_v[:, 2 * D:3 * D], preferred_element_type=f32)
        vmax = jnp.maximum(vmax, jnp.max(jnp.abs(v).reshape(RB // 8, 8, D), axis=0))
        vt = v.T
        zeros8 = jnp.zeros((8, RB), f32)
        onehot = jnp.where(row8 == 0, 1.0, 0.0).astype(f32)
        for h in range(H):
            if h % 2 == 0:
                base = 20 * h
                w = jnp.concatenate([vt[base:base + 16], jnp.where(row8 < 4, vt[base + 16:base + 24], jnp.where(row8 == 4, 1.0, 0.0)), zeros8], axis=0)
            else:
                base = 20 * h - 4
                w = jnp.concatenate([jnp.where(row8 >= 4, vt[base:base + 8], onehot), vt[base + 8:base + 24], zeros8], axis=0)
            vt_s[h, :, pl.ds(off, RB)] = w.astype(bf16)
        return qmax, kmax, vmax

    z = jnp.zeros((8, D), f32)
    qmax, kmax, vmax = lax.fori_loop(0, nrb, proj_body, (z, z, z))
    qm = jnp.max(qmax, axis=0, keepdims=True)
    km = jnp.max(kmax, axis=0, keepdims=True)
    bound = jnp.max(qm * km) * float(DH)
    vm = jnp.max(vmax)
    safe = jnp.logical_and(bound <= SAFE_LOG2, jnp.logical_and(vm <= 2.0 ** 60, vm >= 2.0 ** -50))

    cp_w1.wait(); cp_w2.wait(); cp_wo.wait()

    laneq = lax.broadcasted_iota(jnp.int32, (NQ, 128), 1)
    rowq = lax.broadcasted_iota(jnp.int32, (8, NQ), 0)

    def head_acc(h, qoff, fast):
        start = (20 * h) % 128
        t = (20 * h) // 128
        e = jnp.where(start > 108, t + 5, t) if not isinstance(h, int) else (t + 5 if start > 108 else t)
        mask = ((laneq - start) & 127) < DH
        qm_ = jnp.where(mask, q_s[e, pl.ds(qoff, NQ), :], jnp.zeros((), bf16))
        st = lax.dot_general(k_s[e], qm_, NT, preferred_element_type=f32)
        if not fast:
            st = st - jnp.max(st, axis=0, keepdims=True)
        p = jnp.exp2(st).astype(bf16)
        return jnp.dot(vt_s[h], p, preferred_element_type=f32)

    def head_pair(p, qoff, fast):
        ae = head_acc(2 * p, qoff, fast)
        ao = head_acc(2 * p + 1, qoff, fast)
        ie = 1.0 / ae[20:21, :]
        io = 1.0 / ao[0:1, :]
        oe = ae[0:24] * ie
        oo = ao[0:24] * io
        res = jnp.concatenate([oe[0:16], jnp.where(rowq < 4, oe[16:24], oo[0:8]), oo[8:24]], axis=0)
        if isinstance(p, int):
            ot_s[40 * p:40 * p + 40, :] = res
        else:
            ot_s[pl.ds(pl.multiple_of(40 * p, 8), 40), :] = res

    def attn(qoff, fast, hb):
        npairs = hb // 2
        def body(j, _):
            for pp in range(npairs):
                head_pair(j * npairs + pp, qoff, fast)
            return 0
        if hb == H:
            body(0, 0)
        else:
            lax.fori_loop(0, H // hb, body, 0)

    nqb = S // NQ

    def out_copy(qb, slot):
        return pltpu.make_async_copy(ob_s.at[slot], out_hbm.at[pl.ds(pl.multiple_of(qb * NQ, NQ), NQ)], osem.at[slot])

    def qblock(qb, _):
        qoff = pl.multiple_of(qb * NQ, NQ)

        @pl.when(safe)
        def _():
            attn(qoff, True, HB)

        @pl.when(jnp.logical_not(safe))
        def _():
            attn(qoff, False, 2)

        xb = x_v[pl.ds(qoff, NQ), :]
        o = ot_s[...].T.astype(bf16)
        a = jnp.dot(o, wo_v[...], preferred_element_type=f32)
        hh = jnp.dot(xb, w1_v[...], preferred_element_type=f32) + b1_ref[...].astype(f32)
        act = _mish(hh).astype(bf16)
        b = jnp.dot(act, w2_v[...], preferred_element_type=f32)
        prod = (xb * gw_ref[...]).astype(f32)
        g = jax.nn.sigmoid(jnp.sum(prod, axis=-1, keepdims=True).astype(bf16).astype(f32))
        res = g * a + (1.0 - g) * b
        slot = qb % 2

        @pl.when(qb >= 2)
        def _():
            out_copy(qb - 2, slot).wait()
        ob_s[slot] = res.astype(bf16)
        out_copy(qb, slot).start()
        return 0

    lax.fori_loop(0, nqb, qblock, 0)
    out_copy(nqb - 2, nqb % 2).wait()
    out_copy(nqb - 1, (nqb - 1) % 2).wait()


@jax.jit
def pallas_gated_mix__mha_block__dense_activation_mish__prompt_kernel(
        A_x, A_wqkv, A_wo, B_x, B_w1, B_b1, B_w2, gate_w):
    del B_x
    f32, bf16 = jnp.float32, jnp.bfloat16
    any_spec = pl.BlockSpec(memory_space=pl.ANY)
    out = pl.pallas_call(
        kernel,
        out_shape=jax.ShapeDtypeStruct((S, D), bf16),
        in_specs=[any_spec, any_spec, any_spec, any_spec,
                  pl.BlockSpec(memory_space=pltpu.VMEM), any_spec,
                  pl.BlockSpec(memory_space=pltpu.VMEM)],
        out_specs=any_spec,
        scratch_shapes=[
            pltpu.VMEM((S, D), bf16),
            pltpu.VMEM((D, 3 * D), bf16),
            pltpu.VMEM((D, D), bf16),
            pltpu.VMEM((D, F), bf16),
            pltpu.VMEM((F, D), bf16),
            pltpu.VMEM((9, S, 128), bf16),
            pltpu.VMEM((9, S, 128), bf16),
            pltpu.VMEM((H, 32, S), bf16),
            pltpu.VMEM((D, NQ), f32),
            pltpu.VMEM((2, NQ, D), bf16),
            pltpu.SemaphoreType.DMA((S // RB + 4,)),
            pltpu.SemaphoreType.DMA((2,)),
        ],
        compiler_params=pltpu.CompilerParams(vmem_limit_bytes=100 * 1024 * 1024),
    )(A_x.reshape(S, D), A_wqkv, A_wo, B_w1, B_b1.reshape(1, F), B_w2, gate_w.reshape(1, D))
    return out.reshape(1, S, D)
```

```python
import jax
import jax.numpy as jnp
from jax import lax
from jax.experimental import pallas as pl
from jax.experimental.pallas import tpu as pltpu


S, D, H, DH, F = 2048, 640, 32, 20, 1536
NQ = 512
RB = 512
HB = 8
KC = 128
LAG = 2
FPOS = 127
NBODY = H // HB
FC = F // NBODY
LOG2E = 1.4426950408889634
QSCALE = DH ** -0.5 * LOG2E
SAFE_LOG2 = 48.0


def _mish(h):
    e = jnp.exp(jnp.minimum(h, 20.0))
    n = e * (e + 2.0)
    return h * n / (n + 2.0)


def kernel(x_hbm, wqkv_hbm, wo_hbm, w1_hbm, b1_ref, w2_hbm, gw_ref, out_hbm,
           x_v, wqkv_v, wo_v, w1_v, w2_v, k_s, qt_s, vt_s, ot_s, b_s, b1_s, g_s, ob_s, sems, osem):
    f32, bf16 = jnp.float32, jnp.bfloat16
    nrb = S // RB

    def cp_x(i):
        off = pl.multiple_of(i * RB, RB)
        return pltpu.make_async_copy(x_hbm.at[pl.ds(off, RB)], x_v.at[pl.ds(off, RB)], sems.at[i])

    cp_wqkv = pltpu.make_async_copy(wqkv_hbm, wqkv_v, sems.at[nrb])
    cp_w1 = pltpu.make_async_copy(w1_hbm, w1_v, sems.at[nrb + 1])
    cp_w2 = pltpu.make_async_copy(w2_hbm, w2_v, sems.at[nrb + 2])
    cp_wo = pltpu.make_async_copy(wo_hbm, wo_v, sems.at[nrb + 3])
    cp_x(0).start()
    cp_wqkv.start()
    for i in range(1, nrb):
        cp_x(i).start()
    cp_w1.start(); cp_w2.start(); cp_wo.start()

    lane = lax.broadcasted_iota(jnp.int32, (RB, 128), 1)
    rowt = lax.broadcasted_iota(jnp.int32, (128, RB), 0)
    row8 = lax.broadcasted_iota(jnp.int32, (8, RB), 0)

    gw = gw_ref[...].reshape(1, D)
    b1_s[...] = jnp.broadcast_to(b1_ref[...].reshape(1, F).astype(f32), (8, F))

    def proj_body(i, carry):
        qmax, kmax, vmax = carry
        off = pl.multiple_of(i * RB, RB)
        cp_x(i).wait()
        xb = x_v[pl.ds(off, RB), :]

        v = jnp.dot(xb, wqkv_v[:, 2 * D:3 * D], preferred_element_type=f32).astype(bf16).astype(f32)
        vmax = jnp.maximum(vmax, jnp.max(jnp.abs(v).reshape(RB // 8, 8, D), axis=0))
        vt = v.T
        onehot = jnp.where(row8 == 0, 1.0, 0.0).astype(f32)
        for h in range(H):
            if h % 2 == 0:
                base = 20 * h
                w = jnp.concatenate([vt[base:base + 16], jnp.where(row8 < 4, vt[base + 16:base + 24], jnp.where(row8 == 4, 1.0, 0.0))], axis=0)
            else:
                base = 20 * h - 4
                w = jnp.concatenate([jnp.where(row8 >= 4, vt[base:base + 8], onehot), vt[base + 8:base + 24]], axis=0)
            vt_s[h, :, pl.ds(off, RB)] = w

        prod = (xb * gw).astype(f32)
        gsum = jnp.sum(prod, axis=-1, keepdims=True).astype(bf16).astype(f32)
        g = jax.nn.sigmoid(gsum).astype(bf16).astype(f32)
        g_s[pl.ds(off, RB), :] = jnp.broadcast_to(g, (RB, 128))

        q = (jnp.dot(xb, wqkv_v[:, 0:D], preferred_element_type=f32) * QSCALE).astype(bf16).astype(f32)
        qmax = jnp.maximum(qmax, jnp.max(jnp.abs(q).reshape(RB // 8, 8, D), axis=0))
        qt = q.T
        qtt = [qt[128 * t:128 * (t + 1)] for t in range(5)]
        qtt = qtt + [jnp.where(rowt >= 64, qtt[t], qtt[t + 1]) for t in range(4)]
        for t, tile in enumerate(qtt):
            qt_s[t, :, pl.ds(off, RB)] = tile.astype(bf16)

        k = jnp.dot(xb, wqkv_v[:, D:2 * D], preferred_element_type=f32)
        kb = k.astype(bf16)
        kt = [kb[:, 128 * t:128 * (t + 1)] for t in range(5)]
        kt = kt + [jnp.where(lane >= 64, kt[t], kt[t + 1]) for t in range(4)]
        for t, tile in enumerate(kt):
            k_s[t, pl.ds(off, RB), :] = tile
        kmax = jnp.maximum(kmax, jnp.max(jnp.abs(kb.astype(f32)).reshape(RB // 8, 8, D), axis=0))
        return qmax, kmax, vmax

    cp_wqkv.wait()
    z = jnp.zeros((8, D), f32)
    qmax, kmax, vmax = lax.fori_loop(0, nrb, proj_body, (z, z, z))
    qm = jnp.max(qmax, axis=0, keepdims=True)
    km = jnp.max(kmax, axis=0, keepdims=True)
    bound = jnp.max(qm * km) * float(DH)
    vm = jnp.max(vmax)
    safe = jnp.logical_and(bound <= SAFE_LOG2, jnp.logical_and(vm <= 2.0 ** 60, vm >= 2.0 ** -50))

    cp_w1.wait(); cp_w2.wait(); cp_wo.wait()

    rowm = lax.broadcasted_iota(jnp.int32, (128, NQ), 0)
    rowq = lax.broadcasted_iota(jnp.int32, (8, NQ), 0)

    def head_q(h, qoff):
        start = (20 * h) % 128
        t = (20 * h) // 128
        e = jnp.where(start > 108, t + 5, t)
        mask = ((rowm - start) & 127) < DH
        return e, jnp.where(mask, qt_s[e, :, pl.ds(qoff, NQ)], jnp.zeros((), bf16))

    def store_pair(p, ae, ao):
        ie = 1.0 / ae[20:21, :]
        io = 1.0 / ao[0:1, :]
        oe = ae * ie
        oo = ao * io
        res = jnp.concatenate([oe[0:16], jnp.where(rowq < 4, oe[16:24], oo[0:8]), oo[8:24]], axis=0)
        ot_s[pl.ds(pl.multiple_of(40 * p, 8), 40), :] = res

    def ffn_chunk(j, qoff):
        coff = pl.multiple_of(j * FC, 128)
        xb = x_v[pl.ds(qoff, NQ), :]
        hh = jnp.dot(xb, w1_v[:, pl.ds(coff, FC)], preferred_element_type=f32) + b1_s[0:1, pl.ds(coff, FC)]
        act = _mish(hh).astype(bf16)
        c = jnp.dot(act, w2_v[pl.ds(coff, FC), :], preferred_element_type=f32)
        b_s[...] = jnp.where(j > 0, b_s[...], 0.0) + c

    def fast_body(j, qoff):
        nkc = S // KC
        seq = [(hh, c) for hh in range(HB) for c in range(nkc)]
        qs, ps, accs = {}, {}, {}

        def qk(hh, c):
            if c == 0:
                qs[hh] = head_q(j * HB + hh, qoff)
            e, qm_ = qs[hh]
            st = jnp.dot(k_s[e, c * KC:(c + 1) * KC, :], qm_, preferred_element_type=f32)
            ps[(hh, c)] = jnp.exp2(st).astype(bf16)

        def pv(hh, c):
            r = jnp.dot(vt_s[j * HB + hh, :, c * KC:(c + 1) * KC], ps.pop((hh, c)), preferred_element_type=f32)
            accs[hh] = r if c == 0 else accs[hh] + r
            if c == nkc - 1 and hh % 2 == 1:
                store_pair(j * (HB // 2) + hh // 2, accs.pop(hh - 1), accs.pop(hh))

        for i in range(len(seq) + LAG):
            if i == FPOS:
                ffn_chunk(j, qoff)
            if i < len(seq):
                qk(*seq[i])
            if i - LAG >= 0:
                pv(*seq[i - LAG])

    def slow_head(h, qoff):
        e, qm_ = head_q(h, qoff)
        st = jnp.dot(k_s[e], qm_, preferred_element_type=f32)
        st = st - jnp.max(st, axis=0, keepdims=True)
        p = jnp.exp2(st).astype(bf16)
        return jnp.dot(vt_s[h], p, preferred_element_type=f32)

    nqb = S // NQ

    def out_copy(qb, slot):
        return pltpu.make_async_copy(ob_s.at[slot], out_hbm.at[pl.ds(pl.multiple_of(qb * NQ, NQ), NQ)], osem.at[slot])

    def out_section(qb, qoff):
        o = ot_s[...].T.astype(bf16)
        a = jnp.dot(o, wo_v[...], preferred_element_type=f32)
        g = g_s[pl.ds(qoff, NQ), :]
        g = jnp.concatenate([g] * 5, axis=1)
        res = g * a + (1.0 - g) * b_s[...]
        slot = qb % 2

        @pl.when(qb >= 2)
        def _():
            out_copy(qb - 2, slot).wait()
        ob_s[slot] = res.astype(bf16)
        out_copy(qb, slot).start()

    def qblock(qb, _):
        qoff = pl.multiple_of(qb * NQ, NQ)

        @pl.when(safe)
        def _():
            def body(j, _):
                fast_body(j, qoff)
                return 0
            lax.fori_loop(0, NBODY, body, 0)

        @pl.when(jnp.logical_not(safe))
        def _():
            def body(p, _):
                store_pair(p, slow_head(2 * p, qoff), slow_head(2 * p + 1, qoff))
                return 0
            lax.fori_loop(0, H // 2, body, 0)

            def body2(j, _):
                ffn_chunk(j, qoff)
                return 0
            lax.fori_loop(0, NBODY, body2, 0)

        out_section(qb, qoff)
        return 0

    lax.fori_loop(0, nqb, qblock, 0)
    out_copy(nqb - 2, nqb % 2).wait()
    out_copy(nqb - 1, (nqb - 1) % 2).wait()


@jax.jit
def pallas_gated_mix__mha_block__dense_activation_mish__prompt_kernel(
        A_x, A_wqkv, A_wo, B_x, B_w1, B_b1, B_w2, gate_w):
    del B_x
    f32, bf16 = jnp.float32, jnp.bfloat16
    any_spec = pl.BlockSpec(memory_space=pl.ANY)
    out = pl.pallas_call(
        kernel,
        out_shape=jax.ShapeDtypeStruct((S, D), bf16),
        in_specs=[any_spec, any_spec, any_spec, any_spec,
                  pl.BlockSpec(memory_space=pltpu.VMEM), any_spec,
                  pl.BlockSpec(memory_space=pltpu.VMEM)],
        out_specs=any_spec,
        scratch_shapes=[
            pltpu.VMEM((S, D), bf16),
            pltpu.VMEM((D, 3 * D), bf16),
            pltpu.VMEM((D, D), bf16),
            pltpu.VMEM((D, F), bf16),
            pltpu.VMEM((F, D), bf16),
            pltpu.VMEM((9, S, 128), bf16),
            pltpu.VMEM((9, 128, S), bf16),
            pltpu.VMEM((H, 24, S), f32),
            pltpu.VMEM((D, NQ), f32),
            pltpu.VMEM((NQ, D), f32),
            pltpu.VMEM((8, F), f32),
            pltpu.VMEM((S, 128), f32),
            pltpu.VMEM((2, NQ, D), bf16),
            pltpu.SemaphoreType.DMA((S // RB + 4,)),
            pltpu.SemaphoreType.DMA((2,)),
        ],
        compiler_params=pltpu.CompilerParams(vmem_limit_bytes=100 * 1024 * 1024),
    )(A_x.reshape(S, D), A_wqkv, A_wo, B_w1, B_b1, B_w2, gate_w)
    return out.reshape(1, S, D)
```

```python
import functools
import jax
import jax.numpy as jnp
from jax import lax
from jax.experimental import pallas as pl
from jax.experimental.pallas import tpu as pltpu

S, D, H, DH, F = 2048, 640, 32, 20, 1536
NQ = 512
RB = 256
RB0 = 512
HB = 16
KC = 128
LAG = 2
NBODY = H // HB
FPOS = HB * (S // KC) - 1
FT = 256
FC = (F - FT) // NBODY
KS = 128
OSPLIT = 4
LOG2E = 1.4426950408889634
QSCALE = DH ** -0.5 * LOG2E
L_LO, L_HI = 2.0 ** -60, 2.0 ** 80
V_LO, V_HI = 2.0 ** -30, 2.0 ** 46


def _mish(h):
    e = jnp.exp(jnp.minimum(h, 20.0))
    n = e * (e + 2.0)
    return h * n / (n + 2.0)


def kernel(x_hbm, wqkv_hbm, wo_hbm, w1_hbm, b1_ref, w2_hbm, gw_ref, out_hbm,
           x_v, wqkv_v, wo_v, w1_v, w2_v, k_s, qt_s, vt_s, ot_s, b_s, b1_s, g_s, ob_s, oacc_s, bad_s, redo_s, sems, osem):
    f32, bf16 = jnp.float32, jnp.bfloat16
    nrb = (S - RB0) // RB + 1

    def cp_x(i):
        if isinstance(i, int) and i == 0:
            return pltpu.make_async_copy(x_hbm.at[pl.ds(0, RB0)], x_v.at[pl.ds(0, RB0)], sems.at[0])
        off = pl.multiple_of(RB0 + (i - 1) * RB, RB)
        return pltpu.make_async_copy(x_hbm.at[pl.ds(off, RB)], x_v.at[pl.ds(off, RB)], sems.at[i])

    cp_wv = pltpu.make_async_copy(wqkv_hbm.at[:, pl.ds(2 * D, D)], wqkv_v.at[:, pl.ds(2 * D, D)], sems.at[nrb])
    cp_wqk = pltpu.make_async_copy(wqkv_hbm.at[:, pl.ds(0, 2 * D)], wqkv_v.at[:, pl.ds(0, 2 * D)], sems.at[nrb + 4])
    cp_w1 = pltpu.make_async_copy(w1_hbm, w1_v, sems.at[nrb + 1])
    cp_w2 = pltpu.make_async_copy(w2_hbm, w2_v, sems.at[nrb + 2])
    cp_wo = pltpu.make_async_copy(wo_hbm, wo_v, sems.at[nrb + 3])
    cp_x(0).start()
    cp_wv.start()
    cp_wqk.start()
    for i in range(1, nrb):
        cp_x(i).start()
    cp_w1.start(); cp_w2.start(); cp_wo.start()

    gw = gw_ref[...].reshape(1, D)
    b1_s[...] = jnp.broadcast_to(b1_ref[...].reshape(1, F).astype(f32), (8, F))

    def proj_body(i, carry, first=False):
        vmax = carry
        rb = RB0 if first else RB
        off = 0 if first else pl.multiple_of(RB0 + (i - 1) * RB, RB)
        lane = lax.broadcasted_iota(jnp.int32, (rb, 128), 1)
        rowt = lax.broadcasted_iota(jnp.int32, (128, rb), 0)
        row8 = lax.broadcasted_iota(jnp.int32, (8, rb), 0)
        cp_x(i).wait()
        xb = x_v[pl.ds(off, rb), :]

        v = jnp.dot(xb, wqkv_v[:, 2 * D:3 * D], preferred_element_type=f32)
        if first:
            cp_wqk.wait()
            xb = x_v[pl.ds(off, rb), :]
            q = jnp.dot(xb, wqkv_v[:, 0:D], preferred_element_type=f32)
        v = v.astype(bf16).astype(f32)
        vmax = jnp.maximum(vmax, jnp.max(jnp.abs(v).reshape(rb // 8, 8, D), axis=0))
        vt = v.T
        onehot = jnp.where(row8 == 0, 1.0, 0.0).astype(f32)
        for h in range(H):
            if h % 2 == 0:
                base = 20 * h
                w = jnp.concatenate([vt[base:base + 16], jnp.where(row8 < 4, vt[base + 16:base + 24], jnp.where(row8 == 4, 1.0, 0.0))], axis=0)
            else:
                base = 20 * h - 4
                w = jnp.concatenate([jnp.where(row8 >= 4, vt[base:base + 8], onehot), vt[base + 8:base + 24]], axis=0)
            vt_s[h, :, pl.ds(off, rb)] = w

        prod = (xb * gw).astype(f32)
        gsum = jnp.sum(prod, axis=-1, keepdims=True).astype(bf16).astype(f32)
        g = jax.nn.sigmoid(gsum).astype(bf16).astype(f32)
        g_s[pl.ds(off, rb), :] = jnp.broadcast_to(g, (rb, 128))

        if not first:
            q = jnp.dot(xb, wqkv_v[:, 0:D], preferred_element_type=f32)
        q = (q * QSCALE).astype(bf16).astype(f32)
        qt = q.T
        qtt = [qt[128 * t:128 * (t + 1)] for t in range(5)]
        qtt = qtt + [jnp.where(rowt >= 64, qtt[t], qtt[t + 1]) for t in range(4)]
        for t, tile in enumerate(qtt):
            qt_s[t, :, pl.ds(off, rb)] = tile.astype(bf16)

        k = jnp.dot(xb, wqkv_v[:, D:2 * D], preferred_element_type=f32)
        kb = k.astype(bf16)
        kt = [kb[:, 128 * t:128 * (t + 1)] for t in range(5)]
        kt = kt + [jnp.where(lane >= 64, kt[t], kt[t + 1]) for t in range(4)]
        for t, tile in enumerate(kt):
            k_s[t, pl.ds(off, rb), :] = tile
        return vmax

    cp_wv.wait()
    z = jnp.zeros((8, D), f32)
    vmax = lax.fori_loop(1, nrb, proj_body, proj_body(0, z, first=True))

    cp_w1.wait(); cp_w2.wait(); cp_wo.wait()

    rowm = lax.broadcasted_iota(jnp.int32, (128, NQ), 0)
    rowq = lax.broadcasted_iota(jnp.int32, (8, NQ), 0)

    def head_q(h, qoff):
        start = (20 * h) % 128
        t = (20 * h) // 128
        e = jnp.where(start > 108, t + 5, t)
        mask = ((rowm - start) & 127) < DH
        return e, jnp.where(mask, qt_s[e, :, pl.ds(qoff, NQ)], jnp.zeros((), bf16))

    def store_pair(p, ae, ao, check=False):
        le, lo = ae[20:21, :], ao[0:1, :]
        bad = None
        if check:
            ok = (le >= L_LO) & (le <= L_HI) & (lo >= L_LO) & (lo <= L_HI)
            bad = jnp.where(ok, 0.0, 1.0)
            bad = functools.reduce(jnp.maximum, [bad[:, 128 * t:128 * (t + 1)] for t in range(NQ // 128)])
        ie = 1.0 / le
        io = 1.0 / lo
        oe = ae * ie
        oo = ao * io
        res = jnp.concatenate([oe[0:16], jnp.where(rowq < 4, oe[16:24], oo[0:8]), oo[8:24]], axis=0)
        ot_s[pl.ds(pl.multiple_of(40 * p, 8), 40), :] = res
        return bad

    def ffn_cols(coff, width, qoff):
        xb = x_v[pl.ds(qoff, NQ), :]
        hh = jnp.dot(xb, w1_v[:, pl.ds(coff, width)], preferred_element_type=f32) + b1_s[0:1, pl.ds(coff, width)]
        act = _mish(hh).astype(bf16)
        return act

    def ffn_chunk(j, qoff, width=FC):
        coff = pl.multiple_of(j * width, 128)
        act = ffn_cols(coff, width, qoff)
        c = jnp.dot(act, w2_v[pl.ds(coff, width), :], preferred_element_type=f32)
        b_s[...] = jnp.where(j > 0, b_s[...], 0.0) + c

    def fast_body(j, qb, qoff):
        nkc = S // KC
        seq = [(hh, c) for hh in range(HB) for c in range(nkc)]
        qs, ps, accs, bads = {}, {}, {}, []

        def qk(hh, c):
            if c == 0:
                qs[hh] = head_q(j * HB + hh, qoff)
            e, qm_ = qs[hh]
            st = jnp.dot(k_s[e, c * KC:(c + 1) * KC, :], qm_, preferred_element_type=f32)
            ps[(hh, c)] = jnp.exp2(st).astype(bf16)

        def pv(hh, c):
            r = jnp.dot(vt_s[j * HB + hh, :, c * KC:(c + 1) * KC], ps.pop((hh, c)), preferred_element_type=f32)
            accs[hh] = r if c == 0 else accs[hh] + r
            if c == nkc - 1 and hh % 2 == 1:
                bads.append(store_pair(j * (HB // 2) + hh // 2, accs.pop(hh - 1), accs.pop(hh), check=True))

        for i in range(len(seq) + LAG):
            if i == FPOS:
                ffn_chunk(j, qoff)
            if i < len(seq):
                qk(*seq[i])
            if i - LAG >= 0:
                pv(*seq[i - LAG])
        bad_s[qb * NBODY + j] = jnp.broadcast_to(functools.reduce(jnp.maximum, bads), (8, 128))

    def slow_attention(qoff):
        def hbody(h, _):
            e, qm_ = head_q(h, qoff)

            def scores(c):
                return jnp.dot(k_s[e, pl.ds(pl.multiple_of(c * KS, KS), KS), :], qm_, preferred_element_type=f32)

            def p1(c, m8):
                return jnp.maximum(m8, jnp.max(scores(c).reshape(KS // 8, 8, NQ), axis=0))
            m = jnp.max(lax.fori_loop(0, S // KS, p1, jnp.full((8, NQ), -jnp.inf, f32)), axis=0, keepdims=True)

            def p2(c, acc):
                p = jnp.exp2(scores(c) - m).astype(bf16)
                return acc + jnp.dot(vt_s[h, :, pl.ds(pl.multiple_of(c * KS, KS), KS)], p, preferred_element_type=f32)
            oacc_s[h] = lax.fori_loop(0, S // KS, p2, jnp.zeros((24, NQ), f32))
            return 0
        lax.fori_loop(0, H, hbody, 0)

        def cbody(p, _):
            store_pair(p, oacc_s[2 * p], oacc_s[2 * p + 1])
            return 0
        lax.fori_loop(0, H // 2, cbody, 0)

    nqb = S // NQ

    OM = NQ // OSPLIT

    def out_copy(qb, slot, r):
        return pltpu.make_async_copy(ob_s.at[slot, pl.ds(r * OM, OM)],
                                     out_hbm.at[pl.ds(pl.multiple_of(qb * NQ + r * OM, OM), OM)], osem.at[slot, r])

    def out_section(qb, qoff):
        slot = qb % 2

        @pl.when(qb >= 2)
        def _():
            for r in range(OSPLIT):
                out_copy(qb - 2, slot, r).wait()
        act = ffn_cols(F - FT, FT, qoff)
        o = ot_s[...].T.astype(bf16)
        for r in range(OSPLIT):
            rs = slice(r * OM, (r + 1) * OM)
            g = g_s[pl.ds(qoff + r * OM, OM), :]
            for n in range(D // 128):
                cs = slice(128 * n, 128 * (n + 1))
                a = jnp.dot(o[rs], wo_v[:, cs], preferred_element_type=f32)
                bb = b_s[rs, cs] + jnp.dot(act[rs], w2_v[F - FT:F, cs], preferred_element_type=f32)
                ob_s[slot, rs, cs] = (g * a + (1.0 - g) * bb).astype(bf16)
            out_copy(qb, slot, r).start()

    def qblock(qb, attempt):
        qoff = pl.multiple_of(qb * NQ, NQ)

        @pl.when(attempt == 0)
        def _():
            def body(j, _):
                fast_body(j, qb, qoff)
                return 0
            lax.fori_loop(0, NBODY, body, 0)

        @pl.when(attempt != 0)
        def _():
            slow_attention(qoff)

            def body2(t, _):
                j = t // 4
                roff = pl.multiple_of((t % 4) * 128, 128)
                coff = pl.multiple_of(j * 128, 128)
                xb = x_v[pl.ds(qoff + roff, 128), :]
                hh = jnp.dot(xb, w1_v[:, pl.ds(coff, 128)], preferred_element_type=f32) + b1_s[0:1, pl.ds(coff, 128)]
                c = jnp.dot(_mish(hh).astype(bf16), w2_v[pl.ds(coff, 128), :], preferred_element_type=f32)
                b_s[pl.ds(roff, 128), :] = jnp.where(j > 0, b_s[pl.ds(roff, 128), :], 0.0) + c
                return 0
            lax.fori_loop(0, 4 * ((F - FT) // 128), body2, 0)

        out_section(qb, qoff)
        return attempt

    def attempt_body(attempt, _):
        @pl.when(redo_s[0] > 0)
        def _():
            lax.fori_loop(0, nqb, qblock, attempt)

            @pl.when(attempt == 0)
            def _():
                vm = jnp.max(vmax)
                unsafe = jnp.where((vm >= V_LO) & (vm <= V_HI), jnp.max(bad_s[...]), 1.0)
                redo_s[0] = (unsafe > 0.0).astype(jnp.int32)

            for r in range(OSPLIT):
                out_copy(nqb - 2, nqb % 2, r).wait()
            for r in range(OSPLIT):
                out_copy(nqb - 1, (nqb - 1) % 2, r).wait()
        return 0

    redo_s[0] = 1
    lax.fori_loop(0, 2, attempt_body, 0)


@jax.jit
def pallas_gated_mix__mha_block__dense_activation_mish__prompt_kernel(
        A_x, A_wqkv, A_wo, B_x, B_w1, B_b1, B_w2, gate_w):
    del B_x
    f32, bf16 = jnp.float32, jnp.bfloat16
    any_spec = pl.BlockSpec(memory_space=pl.ANY)
    out = pl.pallas_call(
        kernel,
        out_shape=jax.ShapeDtypeStruct((S, D), bf16),
        in_specs=[any_spec, any_spec, any_spec, any_spec,
                  pl.BlockSpec(memory_space=pltpu.VMEM), any_spec,
                  pl.BlockSpec(memory_space=pltpu.VMEM)],
        out_specs=any_spec,
        scratch_shapes=[
            pltpu.VMEM((S, D), bf16),
            pltpu.VMEM((D, 3 * D), bf16),
            pltpu.VMEM((D, D), bf16),
            pltpu.VMEM((D, F), bf16),
            pltpu.VMEM((F, D), bf16),
            pltpu.VMEM((9, S, 128), bf16),
            pltpu.VMEM((9, 128, S), bf16),
            pltpu.VMEM((H, 24, S), f32),
            pltpu.VMEM((D, NQ), f32),
            pltpu.VMEM((NQ, D), f32),
            pltpu.VMEM((8, F), f32),
            pltpu.VMEM((S, 128), f32),
            pltpu.VMEM((2, NQ, D), bf16),
            pltpu.VMEM((H, 24, NQ), f32),
            pltpu.VMEM((S // NQ * NBODY, 8, 128), f32),
            pltpu.SMEM((1,), jnp.int32),
            pltpu.SemaphoreType.DMA(((S - RB0) // RB + 1 + 5,)),
            pltpu.SemaphoreType.DMA((2, OSPLIT)),
        ],
        compiler_params=pltpu.CompilerParams(vmem_limit_bytes=100 * 1024 * 1024),
    )(A_x.reshape(S, D), A_wqkv, A_wo, B_w1, B_b1, B_w2, gate_w)
    return out.reshape(1, S, D)
```

```python
import functools

import jax
import jax.numpy as jnp
from jax import lax
from jax.experimental import pallas as pl
from jax.experimental.pallas import tpu as pltpu

S, D, H, DH, F = 2048, 640, 32, 20, 1536
NQ = 512
RB0, RB = 512, 256
HB = 16
NBODY = H // HB
KC = 128
LAG = 2
FT = 256
FC = (F - FT) // NBODY
OSPLIT = 4
QSCALE = DH ** -0.5 * 1.4426950408889634
L_LO, L_HI = 2.0 ** -60, 2.0 ** 80
V_LO, V_HI = 2.0 ** -30, 2.0 ** 46


def _mish(h):
    e = jnp.exp(jnp.minimum(h, 20.0))
    n = e * (e + 2.0)
    return h * n / (n + 2.0)


def _kernel(x_hbm, wqkv_hbm, wo_hbm, w1_hbm, b1_hbm, w2_hbm, gw_hbm, out_hbm,
            x_v, wqk_v, wv_v, wo_v, w1_v, w2_v, k_s, qt_s, vt_s, ot_s, b_s, b1_s, g_s,
            ob_s, oacc_s, bad_s, b1_v, gw_v, redo_s, sems, osem):
    f32, bf16 = jnp.float32, jnp.bfloat16
    nrb = (S - RB0) // RB + 1
    nqb = S // NQ

    def cp_x(i):
        if isinstance(i, int) and i == 0:
            return pltpu.make_async_copy(x_hbm.at[pl.ds(0, RB0)], x_v.at[pl.ds(0, RB0)], sems.at[0])
        off = pl.multiple_of(RB0 + (i - 1) * RB, RB)
        return pltpu.make_async_copy(x_hbm.at[pl.ds(off, RB)], x_v.at[pl.ds(off, RB)], sems.at[i])

    cp_wv = pltpu.make_async_copy(wqkv_hbm.at[:, pl.ds(2 * D, D)], wv_v, sems.at[nrb])
    cp_w1 = pltpu.make_async_copy(w1_hbm, w1_v, sems.at[nrb + 1])
    cp_w2 = pltpu.make_async_copy(w2_hbm, w2_v, sems.at[nrb + 2])
    cp_wo = pltpu.make_async_copy(wo_hbm, wo_v, sems.at[nrb + 3])
    cp_wqk = pltpu.make_async_copy(wqkv_hbm.at[:, pl.ds(0, 2 * D)], wqk_v, sems.at[nrb + 4])
    cp_gw = pltpu.make_async_copy(gw_hbm, gw_v, sems.at[nrb + 5])
    cp_b1 = pltpu.make_async_copy(b1_hbm, b1_v, sems.at[nrb + 6])
    cp_x(0).start()
    cp_wv.start()
    cp_gw.start()
    cp_b1.start()
    cp_wqk.start()
    for i in range(1, nrb):
        cp_x(i).start()
    cp_w1.start()
    cp_w2.start()
    cp_wo.start()

    def proj_body(i, vmax, first=False):
        rb = RB0 if first else RB
        off = 0 if first else pl.multiple_of(RB0 + (i - 1) * RB, RB)
        lane = lax.broadcasted_iota(jnp.int32, (rb, 128), 1)
        rowt = lax.broadcasted_iota(jnp.int32, (128, rb), 0)
        row8 = lax.broadcasted_iota(jnp.int32, (8, rb), 0)
        cp_x(i).wait()
        xb = x_v[pl.ds(off, rb), :]

        v = jnp.dot(xb, wv_v[...], preferred_element_type=f32)
        if first:
            cp_wqk.wait()
            xb = x_v[pl.ds(off, rb), :]
            q = jnp.dot(xb, wqk_v[:, 0:D], preferred_element_type=f32)
        v = v.astype(bf16).astype(f32)
        vmax = jnp.maximum(vmax, jnp.max(jnp.abs(v).reshape(rb // 8, 8, D), axis=0))
        vt = v.T
        onehot = jnp.where(row8 == 0, 1.0, 0.0).astype(f32)
        for h in range(H):
            if h % 2 == 0:
                base = DH * h
                w = jnp.concatenate(
                    [vt[base:base + 16],
                     jnp.where(row8 < 4, vt[base + 16:base + 24], jnp.where(row8 == 4, 1.0, 0.0))], axis=0)
            else:
                base = DH * h - 4
                w = jnp.concatenate(
                    [jnp.where(row8 >= 4, vt[base:base + 8], onehot), vt[base + 8:base + 24]], axis=0)
            vt_s[h, :, pl.ds(off, rb)] = w

        prod = (xb * gw_v[...].reshape(1, D)).astype(f32)
        gsum = jnp.sum(prod, axis=-1, keepdims=True).astype(bf16).astype(f32)
        g = jax.nn.sigmoid(gsum).astype(bf16).astype(f32)
        g_s[pl.ds(off, rb), :] = jnp.broadcast_to(g, (rb, 128))

        if not first:
            q = jnp.dot(xb, wqk_v[:, 0:D], preferred_element_type=f32)
        q = (q * QSCALE).astype(bf16).astype(f32)
        qt = q.T
        qtt = [qt[128 * t:128 * (t + 1)] for t in range(5)]
        qtt = qtt + [jnp.where(rowt >= 64, qtt[t], qtt[t + 1]) for t in range(4)]
        for t, tile in enumerate(qtt):
            qt_s[t, :, pl.ds(off, rb)] = tile.astype(bf16)

        kb = jnp.dot(xb, wqk_v[:, D:2 * D], preferred_element_type=f32).astype(bf16)
        kt = [kb[:, 128 * t:128 * (t + 1)] for t in range(5)]
        kt = kt + [jnp.where(lane >= 64, kt[t], kt[t + 1]) for t in range(4)]
        for t, tile in enumerate(kt):
            k_s[t, pl.ds(off, rb), :] = tile
        return vmax

    cp_wv.wait()
    cp_gw.wait()
    vmax = proj_body(0, jnp.zeros((8, D), f32), first=True)
    vmax = lax.fori_loop(1, nrb, proj_body, vmax)

    cp_w1.wait()
    cp_w2.wait()
    cp_wo.wait()
    cp_b1.wait()
    b1_s[...] = jnp.broadcast_to(b1_v[...].reshape(1, F).astype(f32), (8, F))

    rowm = lax.broadcasted_iota(jnp.int32, (128, NQ), 0)
    rowq = lax.broadcasted_iota(jnp.int32, (8, NQ), 0)

    def head_q(h, qoff):
        start = (DH * h) % 128
        t = (DH * h) // 128
        e = jnp.where(start > 128 - DH, t + 5, t)
        mask = ((rowm - start) & 127) < DH
        return e, jnp.where(mask, qt_s[e, :, pl.ds(qoff, NQ)], jnp.zeros((), bf16))

    def store_pair(p, ae, ao, check=False):
        le, lo = ae[20:21, :], ao[0:1, :]
        bad = None
        if check:
            ok = (le >= L_LO) & (le <= L_HI) & (lo >= L_LO) & (lo <= L_HI)
            bad = jnp.where(ok, 0.0, 1.0)
            bad = functools.reduce(jnp.maximum, [bad[:, 128 * t:128 * (t + 1)] for t in range(NQ // 128)])
        oe = ae * (1.0 / le)
        oo = ao * (1.0 / lo)
        res = jnp.concatenate([oe[0:16], jnp.where(rowq < 4, oe[16:24], oo[0:8]), oo[8:24]], axis=0)
        ot_s[pl.ds(pl.multiple_of(2 * DH * p, 8), 2 * DH), :] = res
        return bad

    def ffn_act(coff, width, qoff):
        xb = x_v[pl.ds(qoff, NQ), :]
        hh = jnp.dot(xb, w1_v[:, pl.ds(coff, width)], preferred_element_type=f32)
        return _mish(hh + b1_s[0:1, pl.ds(coff, width)]).astype(bf16)

    def fast_body(j, qb, qoff):
        nkc = S // KC
        seq = [(hh, c) for hh in range(HB) for c in range(nkc)]
        qs, ps, accs, bads = {}, {}, {}, []

        def qk(hh, c):
            if c == 0:
                qs[hh] = head_q(j * HB + hh, qoff)
            e, qm = qs[hh]
            st = jnp.dot(k_s[e, c * KC:(c + 1) * KC, :], qm, preferred_element_type=f32)
            ps[(hh, c)] = jnp.exp2(st).astype(bf16)

        def pv(hh, c):
            r = jnp.dot(vt_s[j * HB + hh, :, c * KC:(c + 1) * KC], ps.pop((hh, c)), preferred_element_type=f32)
            accs[hh] = r if c == 0 else accs[hh] + r
            if c == nkc - 1 and hh % 2 == 1:
                bads.append(store_pair(j * (HB // 2) + hh // 2, accs.pop(hh - 1), accs.pop(hh), check=True))

        for i in range(len(seq) + LAG):
            if i == len(seq) - 1:
                coff = pl.multiple_of(j * FC, 128)
                c = jnp.dot(ffn_act(coff, FC, qoff), w2_v[pl.ds(coff, FC), :], preferred_element_type=f32)
                b_s[...] = jnp.where(j > 0, b_s[...], 0.0) + c
            if i < len(seq):
                qk(*seq[i])
            if i >= LAG:
                pv(*seq[i - LAG])
        bad_s[qb * NBODY + j] = jnp.broadcast_to(functools.reduce(jnp.maximum, bads), (8, 128))

    def slow_blocks(qoff):
        def hbody(h, _):
            e, qm = head_q(h, qoff)

            def scores(c):
                return jnp.dot(k_s[e, pl.ds(pl.multiple_of(c * KC, KC), KC), :], qm, preferred_element_type=f32)

            def pmax(c, m8):
                return jnp.maximum(m8, jnp.max(scores(c).reshape(KC // 8, 8, NQ), axis=0))
            m8 = lax.fori_loop(0, S // KC, pmax, jnp.full((8, NQ), -jnp.inf, f32))
            m = jnp.max(m8, axis=0, keepdims=True)

            def pacc(c, acc):
                p = jnp.exp2(scores(c) - m).astype(bf16)
                return acc + jnp.dot(vt_s[h, :, pl.ds(pl.multiple_of(c * KC, KC), KC)], p,
                                     preferred_element_type=f32)
            oacc_s[h] = lax.fori_loop(0, S // KC, pacc, jnp.zeros((24, NQ), f32))
            return 0
        lax.fori_loop(0, H, hbody, 0)

        def cbody(p, _):
            store_pair(p, oacc_s[2 * p], oacc_s[2 * p + 1])
            return 0
        lax.fori_loop(0, H // 2, cbody, 0)

        def fbody(t, _):
            j = t // 4
            roff = pl.multiple_of((t % 4) * 128, 128)
            coff = pl.multiple_of(j * 128, 128)
            xb = x_v[pl.ds(qoff + roff, 128), :]
            hh = jnp.dot(xb, w1_v[:, pl.ds(coff, 128)], preferred_element_type=f32) + b1_s[0:1, pl.ds(coff, 128)]
            c = jnp.dot(_mish(hh).astype(bf16), w2_v[pl.ds(coff, 128), :], preferred_element_type=f32)
            b_s[pl.ds(roff, 128), :] = jnp.where(j > 0, b_s[pl.ds(roff, 128), :], 0.0) + c
            return 0
        lax.fori_loop(0, 4 * ((F - FT) // 128), fbody, 0)

    om = NQ // OSPLIT

    def out_copy(qb, slot, r):
        return pltpu.make_async_copy(
            ob_s.at[slot, pl.ds(r * om, om)],
            out_hbm.at[pl.ds(pl.multiple_of(qb * NQ + r * om, om), om)], osem.at[slot, r])

    def out_section(qb, qoff):
        slot = qb % 2

        @pl.when(qb >= 2)
        def _():
            for r in range(OSPLIT):
                out_copy(qb - 2, slot, r).wait()
        act = ffn_act(F - FT, FT, qoff)
        o = ot_s[...].T.astype(bf16)
        for r in range(OSPLIT):
            rs = slice(r * om, (r + 1) * om)
            g = g_s[pl.ds(qoff + r * om, om), :]
            for n in range(D // 128):
                cs = slice(128 * n, 128 * (n + 1))
                a = jnp.dot(o[rs], wo_v[:, cs], preferred_element_type=f32)
                b = b_s[rs, cs] + jnp.dot(act[rs], w2_v[F - FT:F, cs], preferred_element_type=f32)
                ob_s[slot, rs, cs] = (g * a + (1.0 - g) * b).astype(bf16)
            out_copy(qb, slot, r).start()

    def qblock(qb, attempt):
        qoff = pl.multiple_of(qb * NQ, NQ)

        @pl.when(attempt == 0)
        def _():
            def body(j, _):
                fast_body(j, qb, qoff)
                return 0
            lax.fori_loop(0, NBODY, body, 0)

        @pl.when(attempt != 0)
        def _():
            slow_blocks(qoff)

        out_section(qb, qoff)
        return attempt

    def attempt_body(attempt, _):
        @pl.when(redo_s[0] > 0)
        def _():
            lax.fori_loop(0, nqb, qblock, attempt)

            @pl.when(attempt == 0)
            def _():
                vm = jnp.max(vmax)
                unsafe = jnp.where((vm >= V_LO) & (vm <= V_HI), jnp.max(bad_s[...]), 1.0)
                redo_s[0] = (unsafe > 0.0).astype(jnp.int32)

            for qb in (nqb - 2, nqb - 1):
                for r in range(OSPLIT):
                    out_copy(qb, qb % 2, r).wait()
        return 0

    redo_s[0] = 1
    lax.fori_loop(0, 2, attempt_body, 0)


@jax.jit
def pallas_gated_mix__mha_block__dense_activation_mish__prompt_kernel(
    A_x: jax.Array,
    A_wqkv: jax.Array,
    A_wo: jax.Array,
    B_x: jax.Array,
    B_w1: jax.Array,
    B_b1: jax.Array,
    B_w2: jax.Array,
    gate_w: jax.Array,
):
    del B_x
    f32, bf16 = jnp.float32, jnp.bfloat16
    any_spec = pl.BlockSpec(memory_space=pl.ANY)
    out = pl.pallas_call(
        _kernel,
        out_shape=jax.ShapeDtypeStruct((S, D), bf16),
        in_specs=[any_spec] * 7,
        out_specs=any_spec,
        scratch_shapes=[
            pltpu.VMEM((S, D), bf16),
            pltpu.VMEM((D, 2 * D), bf16),
            pltpu.VMEM((D, D), bf16),
            pltpu.VMEM((D, D), bf16),
            pltpu.VMEM((D, F), bf16),
            pltpu.VMEM((F, D), bf16),
            pltpu.VMEM((9, S, 128), bf16),
            pltpu.VMEM((9, 128, S), bf16),
            pltpu.VMEM((H, 24, S), f32),
            pltpu.VMEM((D, NQ), f32),
            pltpu.VMEM((NQ, D), f32),
            pltpu.VMEM((8, F), f32),
            pltpu.VMEM((S, 128), f32),
            pltpu.VMEM((2, NQ, D), bf16),
            pltpu.VMEM((H, 24, NQ), f32),
            pltpu.VMEM((S // NQ * NBODY, 8, 128), f32),
            pltpu.VMEM((F,), bf16),
            pltpu.VMEM((D,), bf16),
            pltpu.SMEM((1,), jnp.int32),
            pltpu.SemaphoreType.DMA(((S - RB0) // RB + 8,)),
            pltpu.SemaphoreType.DMA((2, OSPLIT)),
        ],
        compiler_params=pltpu.CompilerParams(vmem_limit_bytes=100 * 1024 * 1024),
    )(A_x.reshape(S, D), A_wqkv, A_wo, B_w1, B_b1, B_w2, gate_w)
    return out.reshape(1, S, D)
```
